```python
import jax
import jax.numpy as jnp

def _softmax(x, axis=-1):
    return jax.nn.softmax(x, axis=axis)
def _gelu(x):
    return jax.nn.gelu(x, approximate=True)
def _silu(x):
    return jax.nn.silu(x)
def _sigmoid(x):
    return jax.nn.sigmoid(x)
def _layernorm(x, axis=-1, eps=1e-5):
    m = jnp.mean(x, axis=axis, keepdims=True)
    v = jnp.var(x, axis=axis, keepdims=True)
    return (x - m) / jnp.sqrt(v + eps)
def _scatter_add(tgt, idx, src, axis=0):
    return tgt.at[idx].add(src)
def _segment_sum(src, seg, n):
    return jax.ops.segment_sum(src, seg, n)
class _Rng:
    def __init__(self, key):
        self._k = key
    def _next(self):
        self._k, sub = jax.random.split(self._k)
        return sub
    def normal(self, shape):
        return jax.random.normal(self._next(), shape, dtype=jnp.bfloat16)
    def randint(self, lo, hi, shape):
        return jax.random.randint(self._next(), shape, lo, hi, dtype=jnp.int32)
    def uniform(self, shape, lo=0.0, hi=1.0):
        return jax.random.uniform(self._next(), shape, jnp.bfloat16, lo, hi)
    def permutation(self, n):
        return jax.random.permutation(self._next(), n)


kernel_name = 'concat_heads__mha_block_cached__compressed_kv_cla__decode'

def setup_inputs():
    _rng = _Rng(jax.random.key(int.from_bytes(__import__("os").urandom(4), "little")))
    _w = (lambda a: (lambda t: t.astype(jnp.bfloat16) if jnp.issubdtype(t.dtype, jnp.floating) else t)(jnp.asarray(a)))
    def _A_setup():
        B, Sq, D = 4, 1, 576
        H, Sk, Dh = 32, 4096, 128
        return {
            "x": _w((lambda *s: _rng.normal(s) * 0.05)(B, Sq, D)),
            "k_cache": _w((lambda *s: _rng.normal(s) * 0.05)(B, H, Sk, Dh)),
            "v_cache": _w((lambda *s: _rng.normal(s) * 0.05)(B, H, Sk, Dh)),
            "wq": _w((lambda *s: _rng.normal(s) * 0.05)(D, H * Dh) * (D ** -0.5)),
            "wo": _w((lambda *s: _rng.normal(s) * 0.05)(H * Dh, D) * ((H * Dh) ** -0.5)),
        }
    _A_in = _A_setup()

    def _B_setup():
        B, H, Sq, Sk, D, M = 4, 32, 1, 4096, 128, 576
        Dc = 4 * D
        return {
            "x": _w((lambda *s: _rng.normal(s) * 0.05)(B, Sq, M)),
            "c_kv": _w((lambda *s: _rng.normal(s) * 0.05)(B, Sk, Dc)),
            "w_q": _w((lambda *s: _rng.normal(s) * 0.05)(M, H, D) * (M ** -0.5)),
            "w_uk": _w((lambda *s: _rng.normal(s) * 0.05)(Dc, H, D) * (Dc ** -0.5)),
            "w_uv": _w((lambda *s: _rng.normal(s) * 0.05)(Dc, H, D) * (Dc ** -0.5)),
            "w_o": _w((lambda *s: _rng.normal(s) * 0.05)(H, D, M) * ((H * D) ** -0.5)),
        }
    _B_in = _B_setup()

    return {
        "A_x": _A_in["x"],
        "A_k_cache": _A_in["k_cache"],
        "A_v_cache": _A_in["v_cache"],
        "A_wq": _A_in["wq"],
        "A_wo": _A_in["wo"],
        "B_x": _B_in["x"],
        "B_c_kv": _B_in["c_kv"],
        "B_w_q": _B_in["w_q"],
        "B_w_uk": _B_in["w_uk"],
        "B_w_uv": _B_in["w_uv"],
        "B_w_o": _B_in["w_o"],
    }

def reference(A_x, A_k_cache, A_v_cache, A_wq, A_wo, B_x, B_c_kv, B_w_q, B_w_uk, B_w_uv, B_w_o):
    def _A_ref(x, k_cache, v_cache, wq, wo):
        B, Sq, D = x.shape
        H, Dh = 32, 128
        q = (lambda x, *d: x.transpose(*d))((x @ wq).reshape(B, Sq, H, Dh), 0, 2, 1, 3)
        scores = jnp.einsum("bhqd,bhkd->bhqk", q, k_cache) * (Dh ** -0.5)
        p = _softmax(scores, axis=-1)
        o = jnp.einsum("bhqk,bhkd->bhqd", p, v_cache)
        return (lambda x, *d: x.transpose(*d))(o, 0, 2, 1, 3).reshape(B, Sq, H * Dh) @ wo

    def _B_ref(x, c_kv, w_q, w_uk, w_uv, w_o):
        B, Sq, M = x.shape[0], x.shape[1], x.shape[2]
        Sk = c_kv.shape[1]
        H, D = w_q.shape[1], w_q.shape[2]
        q = jnp.einsum("bqm,mhd->bhqd", x, w_q)
        k = jnp.einsum("bkc,chd->bhkd", c_kv, w_uk)
        v = jnp.einsum("bkc,chd->bhkd", c_kv, w_uv)
        scores = jnp.einsum("bhqd,bhkd->bhqk", q, k) * (D ** -0.5)
        off = Sk - Sq
        qi = jnp.arange(Sq)[:, None]
        kj = jnp.arange(Sk)[None, :]
        cmask = kj <= (qi + off)
        scores = jnp.where(cmask[None, None], scores, -1e9)
        p = _softmax(scores, axis=-1)
        ctx = jnp.einsum("bhqk,bhkd->bhqd", p, v)
        return jnp.einsum("bhqd,hdm->bqm", ctx, w_o)

    a = _A_ref(A_x, A_k_cache, A_v_cache, A_wq, A_wo)
    b = _B_ref(B_x, B_c_kv, B_w_q, B_w_uk, B_w_uv, B_w_o)
    return jnp.concatenate([a, b], axis=-1)
```

```python
import functools
import jax
import jax.numpy as jnp
from jax import lax
import jax.experimental.pallas as pl
import jax.experimental.pallas.tpu as pltpu

B, H, SK, DH, DM, DC = 4, 32, 4096, 128, 576, 512
NSTEP = B * H
F32 = jnp.float32
BF16 = jnp.bfloat16
NT = (((1,), (1,)), ((), ()))
SCALE = float(DH) ** -0.5


def _dot(a, b):
    return jnp.dot(a, b, preferred_element_type=F32)


def _dot_nt(a, b):
    return lax.dot_general(a, b, NT, preferred_element_type=F32)


def make_kernel(D=8, B_DMA_STEP=2, B_PIECES=(14, 18, 22, 26, 30, 34, 38, 42)):
    def kernel(xa_h, k_h, v_h, wqa_h, woa_h, xb_h, ckv_h, wqb_h, wuk_h, wuv_h, wob_h,
               o_ref,
               xa_v, xb_v, wqa_v, woa_v, wqb_v, wuk_v, wuv_v, wob_v, ckv_v,
               kbuf, vbuf, qh_s, oh_s, acc_s, qb_s, qabs_s, ctxc_s, ctx_s,
               wsem, csem, ksem, vsem):
        def kv_copies(i):
            slot = i % D
            h = i // B
            b = i % B
            bh = b * H + h
            return (pltpu.make_async_copy(k_h.at[bh], kbuf.at[slot], ksem.at[slot]),
                    pltpu.make_async_copy(v_h.at[bh], vbuf.at[slot], vsem.at[slot]))

        c_xa = pltpu.make_async_copy(xa_h, xa_v, wsem.at[0])
        c_wqa = pltpu.make_async_copy(wqa_h, wqa_v, wsem.at[1])
        c_woa = pltpu.make_async_copy(woa_h, woa_v, wsem.at[2])
        c_xb = pltpu.make_async_copy(xb_h, xb_v, wsem.at[3])
        c_wqb = pltpu.make_async_copy(wqb_h, wqb_v, wsem.at[4])
        c_wuk = pltpu.make_async_copy(wuk_h, wuk_v, wsem.at[5])
        c_wuv = pltpu.make_async_copy(wuv_h, wuv_v, wsem.at[6])
        c_wob = pltpu.make_async_copy(wob_h, wob_v, wsem.at[7])
        c_ckv = [pltpu.make_async_copy(ckv_h.at[b], ckv_v.at[b], csem.at[b]) for b in range(B)]

        c_xa.start()
        c_xb.start()
        c_wqa.start()
        c_woa.start()
        for i in range(D):
            for c in kv_copies(i):
                c.start()

        def pad8(x):
            return jnp.concatenate([x.astype(F32), jnp.zeros((8 - B, x.shape[1]), F32)], axis=0).astype(BF16)

        c_xa.wait()
        c_xb.wait()
        c_wqa.wait()
        qa = _dot(pad8(xa_v[...]), wqa_v[...])
        qa = qa.astype(BF16).astype(F32)
        for h in range(H):
            qh_s[h] = qa[:, h * DH:(h + 1) * DH]
        acc_s[...] = jnp.zeros_like(acc_s)
        oh_s[...] = jnp.zeros_like(oh_s)
        c_woa.wait()

        def b_dma():
            c_wqb.start()
            c_wuk.start()
            for c in c_ckv:
                c.start()
            c_wuv.start()
            c_wob.start()

        def b_q():
            c_wqb.wait()
            w2 = wqb_v[...].reshape(DM, H * DH)
            qb = _dot(pad8(xb_v[...]), w2)
            qb_s[...] = qb.astype(BF16).astype(F32)

        def b_qabs():
            c_wuk.wait()
            qb = qb_s[...]
            rows = lax.broadcasted_iota(jnp.int32, (H, H * DH), 0)
            cols = lax.broadcasted_iota(jnp.int32, (H, H * DH), 1) // DH
            mask = rows == cols
            parts = []
            for b in range(B):
                qrow = jnp.broadcast_to(qb[b:b + 1, :], (H, H * DH))
                parts.append(jnp.where(mask, qrow, 0.0).astype(BF16))
            qexp = jnp.concatenate(parts, axis=0)
            w2 = wuk_v[...].reshape(DC, H * DH)
            qabs = _dot_nt(qexp, w2)
            qabs_s[...] = qabs.astype(BF16)

        def b_attn(b):
            c_ckv[b].wait()
            c = ckv_v[b]
            q = qabs_s[b * H:(b + 1) * H, :]
            s = _dot_nt(q, c) * SCALE
            m = jnp.max(s, axis=-1, keepdims=True)
            p = jnp.exp(s - m)
            l = jnp.sum(p, axis=-1, keepdims=True)
            ctxc = _dot(p.astype(BF16), c) / l
            ctxc_s[b * H:(b + 1) * H, :] = ctxc.astype(BF16)

        def b_ctx():
            c_wuv.wait()
            w2 = wuv_v[...].reshape(DC, H * DH)
            full = _dot(ctxc_s[...], w2)
            rows = lax.broadcasted_iota(jnp.int32, (H, H * DH), 0)
            cols = lax.broadcasted_iota(jnp.int32, (H, H * DH), 1) // DH
            mask = rows == cols
            parts = []
            for b in range(B):
                blk = jnp.where(mask, full[b * H:(b + 1) * H, :], 0.0)
                parts.append(jnp.sum(blk, axis=0, keepdims=True))
            parts.append(jnp.zeros((8 - B, H * DH), F32))
            ctx_s[...] = jnp.concatenate(parts, axis=0)

        def b_out():
            c_wob.wait()
            ctx = ctx_s[...].astype(BF16)
            ob = jnp.zeros((8, DM), F32)
            for h in range(H):
                ob = ob + _dot_nt(ctx[:, h * DH:(h + 1) * DH], wob_v[h])
            o_ref[:, DM:2 * DM] = ob[0:B, :].astype(o_ref.dtype)

        pieces = [b_q, b_qabs] + [functools.partial(b_attn, b) for b in range(B)] + [b_ctx, b_out]
        assert len(pieces) == len(B_PIECES)

        def step(i, carry):
            slot = i % D
            h = i // B
            b = i % B
            ck, cv = kv_copies(i)
            ck.wait()
            q = qh_s[h].astype(BF16)
            s = _dot_nt(q, kbuf[slot]) * SCALE
            m = jnp.max(s, axis=-1, keepdims=True)
            p = jnp.exp(s - m)
            l = jnp.sum(p, axis=-1, keepdims=True)
            cv.wait()
            o = _dot(p.astype(BF16), vbuf[slot]) / l
            row = lax.broadcasted_iota(jnp.int32, (8, DH), 0)
            oh_s[...] = jnp.where(row == b, o, oh_s[...])

            @pl.when(i + D < NSTEP)
            def _():
                for c in kv_copies(i + D):
                    c.start()

            @pl.when(b == B - 1)
            def _():
                w = woa_v[:, pl.ds(pl.multiple_of(h * DH, DH), DH)]
                acc_s[...] += _dot_nt(oh_s[...].astype(BF16), w)

            @pl.when(i == B_DMA_STEP)
            def _():
                b_dma()

            for st, piece in zip(B_PIECES, pieces):
                @pl.when(i == st)
                def _(piece=piece):
                    piece()
            return carry

        lax.fori_loop(0, NSTEP, step, 0)
        o_ref[:, 0:DM] = acc_s[0:B, :].astype(o_ref.dtype)

    scratch = [
        pltpu.VMEM((B, DM), BF16), pltpu.VMEM((B, DM), BF16),
        pltpu.VMEM((DM, H * DH), BF16), pltpu.VMEM((DM, H * DH), BF16),
        pltpu.VMEM((DM, H, DH), BF16), pltpu.VMEM((DC, H, DH), BF16), pltpu.VMEM((DC, H, DH), BF16),
        pltpu.VMEM((H, DM, DH), BF16), pltpu.VMEM((B, SK, DC), BF16),
        pltpu.VMEM((D, SK, DH), BF16), pltpu.VMEM((D, SK, DH), BF16),
        pltpu.VMEM((H, 8, DH), F32), pltpu.VMEM((8, DH), F32), pltpu.VMEM((8, DM), F32),
        pltpu.VMEM((8, H * DH), F32), pltpu.VMEM((B * H, DC), BF16), pltpu.VMEM((B * H, DC), BF16),
        pltpu.VMEM((8, H * DH), F32),
        pltpu.SemaphoreType.DMA((8,)), pltpu.SemaphoreType.DMA((B,)),
        pltpu.SemaphoreType.DMA((D,)), pltpu.SemaphoreType.DMA((D,)),
    ]
    return kernel, scratch


_KERNEL, _SCRATCH = make_kernel()


@jax.jit
def pallas_concat_heads__mha_block_cached__compressed_kv_cla__decode_kernel(
    A_x: jax.Array,
    A_k_cache: jax.Array,
    A_v_cache: jax.Array,
    A_wq: jax.Array,
    A_wo: jax.Array,
    B_x: jax.Array,
    B_c_kv: jax.Array,
    B_w_q: jax.Array,
    B_w_uk: jax.Array,
    B_w_uv: jax.Array,
    B_w_o: jax.Array,
):
    args = (
        A_x.reshape(B, DM),
        A_k_cache.reshape(B * H, SK, DH),
        A_v_cache.reshape(B * H, SK, DH),
        A_wq,
        A_wo.T,
        B_x.reshape(B, DM),
        B_c_kv,
        B_w_q, B_w_uk, B_w_uv,
        B_w_o.transpose(0, 2, 1),
    )
    out = pl.pallas_call(
        _KERNEL,
        in_specs=[pl.BlockSpec(memory_space=pltpu.HBM)] * 11,
        out_specs=pl.BlockSpec(memory_space=pltpu.VMEM),
        out_shape=jax.ShapeDtypeStruct((B, 2 * DM), BF16),
        scratch_shapes=_SCRATCH,
        compiler_params=pltpu.CompilerParams(vmem_limit_bytes=110 * 1024 * 1024),
    )(*args)
    return out.reshape(B, 1, 2 * DM)
```

```python
import functools
import jax
import jax.numpy as jnp
from jax import lax
import jax.experimental.pallas as pl
import jax.experimental.pallas.tpu as pltpu

B, H, SK, DH, DM, DC = 4, 32, 4096, 128, 576, 512
NSTEP = B * H
F32 = jnp.float32
BF16 = jnp.bfloat16
NT = (((1,), (1,)), ((), ()))
SCALE = float(DH) ** -0.5


def _dot(a, b):
    return jnp.dot(a, b, preferred_element_type=F32)


def _dot_nt(a, b):
    return lax.dot_general(a, b, NT, preferred_element_type=F32)


def make_kernel(NSLOT=3, SUB=128, PK=0, PV=1, PW=1):
    LOOK = NSLOT - 1
    NSUB = SK // SUB

    def kernel(xa_h, k_h, v_h, wqa_h, woa_h, xb_h, ckv_h, wqb_h, wuk_h, wuv_h, wob_h,
               o_ref,
               xa_v, xb_v, wqa_v, woa_v, wqb_v, wuk_v, wuv_v, wob_v, ckv_v,
               kv, qh_s, oh_s, acc_s, qb_s, qabs_s, ctxc_s, ctx_s,
               wsem, csem, ksem, vsem):
        def bh_of(i):
            return lax.rem(i, B) * H + lax.div(i, B)

        def kv_wait(slot):
            pltpu.make_async_copy(kv.at[slot, 0], kv.at[slot, 0], ksem.at[slot]).wait()
            pltpu.make_async_copy(kv.at[slot, 1], kv.at[slot, 1], vsem.at[slot]).wait()

        def issue(slot, bh):
            for t in range(NSUB):
                r = t * SUB
                pltpu.make_async_copy(k_h.at[bh, pl.ds(r, SUB)], kv.at[slot, 0, pl.ds(r, SUB)],
                                      ksem.at[slot]).start(priority=PK)
                pltpu.make_async_copy(v_h.at[bh, pl.ds(r, SUB)], kv.at[slot, 1, pl.ds(r, SUB)],
                                      vsem.at[slot]).start(priority=PV)

        c_xa = pltpu.make_async_copy(xa_h, xa_v, wsem.at[0])
        c_wqa = pltpu.make_async_copy(wqa_h, wqa_v, wsem.at[1])
        c_woa = pltpu.make_async_copy(woa_h, woa_v, wsem.at[2])
        c_xb = pltpu.make_async_copy(xb_h, xb_v, wsem.at[3])
        c_wqb = pltpu.make_async_copy(wqb_h, wqb_v, wsem.at[4])
        c_wuk = pltpu.make_async_copy(wuk_h, wuk_v, wsem.at[5])
        c_wuv = pltpu.make_async_copy(wuv_h, wuv_v, wsem.at[6])
        c_wob = pltpu.make_async_copy(wob_h, wob_v, wsem.at[7])
        c_ckv = [pltpu.make_async_copy(ckv_h.at[b], ckv_v.at[b], csem.at[b]) for b in range(B)]

        for c in [c_xb, c_xa, c_wqb, c_wuk] + c_ckv + [c_wuv, c_wob, c_wqa, c_woa]:
            c.start(priority=PW)
        for i in range(LOOK):
            bh = (i % B) * H + i // B
            pltpu.make_async_copy(k_h.at[bh], kv.at[i, 0], ksem.at[i]).start(priority=PW)
            pltpu.make_async_copy(v_h.at[bh], kv.at[i, 1], vsem.at[i]).start(priority=PW)

        def pad8(x):
            return jnp.concatenate([x.astype(F32), jnp.zeros((8 - B, x.shape[1]), F32)], axis=0).astype(BF16)

        def head_mask():
            rows = lax.broadcasted_iota(jnp.int32, (H, H * DH), 0)
            cols = lax.broadcasted_iota(jnp.int32, (H, H * DH), 1) // DH
            return rows == cols

        G = 8
        NG = H // G
        GW = G * DH

        def gmask():
            rows = lax.broadcasted_iota(jnp.int32, (G, GW), 0)
            cols = lax.broadcasted_iota(jnp.int32, (G, GW), 1) // DH
            return rows == cols

        def q_piece(j, c):
            w = wqb_v[:, pl.ds(pl.multiple_of(j * G, G), G), :].reshape(DM, GW)
            qb_s[:, pl.ds(pl.multiple_of(j * GW, GW), GW)] = _dot(pad8(xb_v[...]), w).astype(BF16).astype(F32)
            return c

        def qabs_piece(j, c):
            qg = qb_s[:, pl.ds(pl.multiple_of(j * GW, GW), GW)]
            mask = gmask()
            parts = [jnp.where(mask, jnp.broadcast_to(qg[b:b + 1, :], (G, GW)), 0.0) for b in range(B)]
            qexp = jnp.concatenate(parts, axis=0).astype(BF16)
            w = wuk_v[:, pl.ds(pl.multiple_of(j * G, G), G), :].reshape(DC, GW)
            res = _dot_nt(qexp, w)
            for b in range(B):
                qabs_s[pl.ds(pl.multiple_of(b * H + j * G, G), G), :] = res[b * G:(b + 1) * G, :].astype(BF16).astype(F32)
            return c

        def attn_piece(b, carry):
            for bb in range(B):
                @pl.when(b == bb)
                def _():
                    c_ckv[bb].wait()
            c = ckv_v[b]
            r = pl.ds(pl.multiple_of(b * H, H), H)
            q = qabs_s[r, :].astype(BF16)
            s = _dot_nt(q, c) * SCALE
            m = jnp.max(s, axis=-1, keepdims=True)
            p = jnp.exp(s - m)
            l = jnp.sum(p, axis=-1, keepdims=True)
            ctxc_s[r, :] = _dot(p.astype(BF16), c) / l
            return carry

        def ctx_piece(j, c):
            lhs = jnp.concatenate([ctxc_s[pl.ds(pl.multiple_of(b * H + j * G, G), G), :] for b in range(B)], axis=0).astype(BF16)
            w = wuv_v[:, pl.ds(pl.multiple_of(j * G, G), G), :].reshape(DC, GW)
            full = _dot(lhs, w)
            mask = gmask()
            parts = [jnp.sum(jnp.where(mask, full[b * G:(b + 1) * G, :], 0.0), axis=0, keepdims=True) for b in range(B)]
            parts.append(jnp.zeros((8 - B, GW), F32))
            ctx_s[:, pl.ds(pl.multiple_of(j * GW, GW), GW)] = jnp.concatenate(parts, axis=0)
            return c

        def out_piece(h, ob):
            return ob + _dot_nt(ctx_s[:, pl.ds(pl.multiple_of(h * DH, DH), DH)].astype(BF16), wob_v[h])

        c_xb.wait()
        c_xa.wait()
        c_wqb.wait()
        lax.fori_loop(0, NG, q_piece, 0)
        c_wuk.wait()
        lax.fori_loop(0, NG, qabs_piece, 0)
        lax.fori_loop(0, B, attn_piece, 0)
        c_wuv.wait()
        lax.fori_loop(0, NG, ctx_piece, 0)
        c_wob.wait()
        ob = lax.fori_loop(0, H, out_piece, jnp.zeros((8, DM), F32), unroll=4)
        o_ref[:, DM:2 * DM] = ob[0:B, :].astype(o_ref.dtype)

        c_wqa.wait()
        qa = _dot(pad8(xa_v[...]), wqa_v[...])
        qa = qa.astype(BF16).astype(F32)
        for h in range(H):
            qh_s[h] = qa[:, h * DH:(h + 1) * DH]
        acc_s[...] = jnp.zeros_like(acc_s)
        oh_s[...] = jnp.zeros_like(oh_s)
        c_woa.wait()

        def step(i, carry, do_issue):
            slot = lax.rem(i, NSLOT)
            h = lax.div(i, B)
            b = lax.rem(i, B)
            if do_issue:
                issue(lax.rem(i + LOOK, NSLOT), bh_of(i + LOOK))
            kv_wait(slot)
            q = qh_s[h].astype(BF16)
            s = _dot_nt(q, kv[slot, 0]) * SCALE
            m = jnp.max(s, axis=-1, keepdims=True)
            p = jnp.exp(s - m)
            l = jnp.sum(p, axis=-1, keepdims=True)
            o = _dot(p.astype(BF16), kv[slot, 1]) / l
            row = lax.broadcasted_iota(jnp.int32, (8, DH), 0)
            oh_s[...] = jnp.where(row == b, o, oh_s[...])

            @pl.when(b == B - 1)
            def _():
                w = woa_v[:, pl.ds(pl.multiple_of(h * DH, DH), DH)]
                acc_s[...] += _dot_nt(oh_s[...].astype(BF16), w)
            return carry

        lax.fori_loop(0, NSTEP - LOOK, functools.partial(step, do_issue=True), 0)
        lax.fori_loop(NSTEP - LOOK, NSTEP, functools.partial(step, do_issue=False), 0)
        o_ref[:, 0:DM] = acc_s[0:B, :].astype(o_ref.dtype)

    scratch = [
        pltpu.VMEM((B, DM), BF16), pltpu.VMEM((B, DM), BF16),
        pltpu.VMEM((DM, H * DH), BF16), pltpu.VMEM((DM, H * DH), BF16),
        pltpu.VMEM((DM, H, DH), BF16), pltpu.VMEM((DC, H, DH), BF16), pltpu.VMEM((DC, H, DH), BF16),
        pltpu.VMEM((H, DM, DH), BF16), pltpu.VMEM((B, SK, DC), BF16),
        pltpu.VMEM((NSLOT, 2, SK, DH), BF16),
        pltpu.VMEM((H, 8, DH), F32), pltpu.VMEM((8, DH), F32), pltpu.VMEM((8, DM), F32),
        pltpu.VMEM((8, H * DH), F32), pltpu.VMEM((B * H, DC), F32), pltpu.VMEM((B * H, DC), F32),
        pltpu.VMEM((8, H * DH), F32),
        pltpu.SemaphoreType.DMA((8,)), pltpu.SemaphoreType.DMA((B,)),
        pltpu.SemaphoreType.DMA((NSLOT,)), pltpu.SemaphoreType.DMA((NSLOT,)),
    ]
    return kernel, scratch


@jax.jit
def pallas_concat_heads__mha_block_cached__compressed_kv_cla__decode_kernel(
    A_x, A_k_cache, A_v_cache, A_wq, A_wo, B_x, B_c_kv, B_w_q, B_w_uk, B_w_uv, B_w_o,
):
    kernel, scratch = make_kernel()
    args = (
        A_x.reshape(B, DM),
        A_k_cache.reshape(B * H, SK, DH),
        A_v_cache.reshape(B * H, SK, DH),
        A_wq,
        A_wo.T,
        B_x.reshape(B, DM),
        B_c_kv,
        B_w_q, B_w_uk, B_w_uv,
        B_w_o.transpose(0, 2, 1),
    )
    out = pl.pallas_call(
        kernel,
        in_specs=[pl.BlockSpec(memory_space=pltpu.HBM)] * 11,
        out_specs=pl.BlockSpec(memory_space=pltpu.VMEM),
        out_shape=jax.ShapeDtypeStruct((B, 2 * DM), BF16),
        scratch_shapes=scratch,
        compiler_params=pltpu.CompilerParams(vmem_limit_bytes=110 * 1024 * 1024, disable_bounds_checks=True),
    )(*args)
    return out.reshape(B, 1, 2 * DM)
```

```python
import functools
import jax
import jax.numpy as jnp
from jax import lax
import jax.experimental.pallas as pl
import jax.experimental.pallas.tpu as pltpu

B, H, SK, DH, DM, DC = 4, 32, 4096, 128, 576, 512
NSTEP = B * H
F32 = jnp.float32
BF16 = jnp.bfloat16
NT = (((1,), (1,)), ((), ()))
SCALE = float(DH) ** -0.5
G = 8
NG = H // G
GW = G * DH
SUB = 128
HALF = SK // 2
ORDER = ("wqb", "wuk", "ckv0", "ckv1", "ckv2", "ckv3", "wuv", "wob", "wqa", "woa")
NUNITS = dict(wqb=144, wuk=128, ckv0=128, ckv1=128, ckv2=128, ckv3=128, wuv=128, wob=128, wqa=144, woa=144)


def _dot(a, b):
    return jnp.dot(a, b, preferred_element_type=F32)


def _dot_nt(a, b):
    return lax.dot_general(a, b, NT, preferred_element_type=F32)


def streams_seq(lo, hi, S):
    n = hi - lo
    bnd = [lo + round(n * k / S) for k in range(S + 1)]
    pos = bnd[:-1]
    seq = []
    while len(seq) < n:
        for s in range(S):
            if pos[s] < bnd[s + 1]:
                seq.append(pos[s])
                pos[s] += 1
    return seq


def make_kernel(NSLOT=3, KVS=6, KVP=(0, 1, 0), BS=2, BP=(0, 1), LASTS=(3, 2), LASTP=(0, 1, 0), KVSEQ=None, KVPRIO=None,
                SEGS=(272, 336, 400, 464, 528, 656, 784, 912, 1040, 1112, 1184, 1328)):
    LOOK = NSLOT - 1
    kv_seq = list(KVSEQ) if KVSEQ is not None else streams_seq(0, 64, KVS)
    kv_prio = list(KVPRIO) if KVPRIO is not None else [KVP[i % len(KVP)] for i in range(64)]
    last_seq = streams_seq(0, 32, LASTS[0]) + streams_seq(32, 48, LASTS[1]) + streams_seq(48, 64, LASTS[1])
    last_prio = [LASTP[i % len(LASTP)] for i in range(64)]

    def kernel(xa_h, k_h, v_h, wqa_h, woa_h, xb_h, ckv_h, wqb_h, wuk_h, wuv_h, wob_h,
               o_ref,
               xa_v, xb_v, wqa_v, woa_v, wqb_v, wuk_v, wuv_v, wob_v, ckv_v,
               kv, qh_s, oh_s, acc_s, qb_s, qabs_s, ctxc_s, ctx_s,
               wsem, csem, kvsem):

        def unit_refs(name, u):
            if name in ("wqb", "wuk", "wuv"):
                s, d, sem = {"wqb": (wqb_h, wqb_v, wsem.at[4]), "wuk": (wuk_h, wuk_v, wsem.at[5]),
                             "wuv": (wuv_h, wuv_v, wsem.at[6])}[name]
                return s.at[pl.ds(u * 4, 4)], d.at[pl.ds(u * 4, 4)], sem
            if name == "wob":
                h, r = u // 4, (u % 4) * 144
                return wob_h.at[h, pl.ds(r, 144)], wob_v.at[h, pl.ds(r, 144)], wsem.at[7]
            if name in ("wqa", "woa"):
                s, d, sem = {"wqa": (wqa_h, wqa_v, wsem.at[1]), "woa": (woa_h, woa_v, wsem.at[2])}[name]
                r, c = (u // 2) * 8, (u % 2) * 2048
                return s.at[pl.ds(r, 8), pl.ds(c, 2048)], d.at[pl.ds(r, 8), pl.ds(c, 2048)], sem
            b = int(name[3])
            return ckv_h.at[b, pl.ds(u * 32, 32)], ckv_v.at[b, pl.ds(u * 32, 32)], csem.at[b]

        prog = []
        for name in ORDER:
            for u in streams_seq(0, NUNITS[name], BS):
                prog.append((name, u))

        def issue(lo, hi):
            for n in range(lo, hi):
                s, d, sem = unit_refs(*prog[n])
                pltpu.make_async_copy(s, d, sem).start(priority=BP[n % len(BP)])

        def kv_issue(slot, bh, seq=kv_seq, prio=kv_prio):
            for c, pr in zip(seq, prio):
                which, r = c >> 5, (c & 31) * SUB
                src = k_h if which == 0 else v_h
                si = 0 if which == 0 else 1 + r // HALF
                pltpu.make_async_copy(src.at[bh, pl.ds(r, SUB)], kv.at[slot, which, pl.ds(r, SUB)],
                                      kvsem.at[slot, si]).start(priority=pr)

        def wait_full(dst, sem):
            pltpu.make_async_copy(dst, dst, sem).wait()

        c_xa = pltpu.make_async_copy(xa_h, xa_v, wsem.at[0])
        c_xb = pltpu.make_async_copy(xb_h, xb_v, wsem.at[3])
        c_xb.start()
        c_xa.start()

        def pad8(x):
            return jnp.concatenate([x.astype(F32), jnp.zeros((8 - B, x.shape[1]), F32)], axis=0).astype(BF16)

        def gmask():
            rows = lax.broadcasted_iota(jnp.int32, (G, GW), 0)
            cols = lax.broadcasted_iota(jnp.int32, (G, GW), 1) // DH
            return rows == cols

        def q_piece(j, c):
            w = wqb_v[:, pl.ds(pl.multiple_of(j * G, G), G), :].reshape(DM, GW)
            qb_s[:, pl.ds(pl.multiple_of(j * GW, GW), GW)] = _dot(pad8(xb_v[...]), w).astype(BF16).astype(F32)
            return c

        def qabs_piece(j, c):
            qg = qb_s[:, pl.ds(pl.multiple_of(j * GW, GW), GW)]
            mask = gmask()
            parts = [jnp.where(mask, jnp.broadcast_to(qg[b:b + 1, :], (G, GW)), 0.0) for b in range(B)]
            qexp = jnp.concatenate(parts, axis=0).astype(BF16)
            w = wuk_v[:, pl.ds(pl.multiple_of(j * G, G), G), :].reshape(DC, GW)
            res = _dot_nt(qexp, w)
            for b in range(B):
                qabs_s[pl.ds(pl.multiple_of(b * H + j * G, G), G), :] = res[b * G:(b + 1) * G, :]
            return c

        def attn_piece(b):
            c = ckv_v[b]
            r = pl.ds(pl.multiple_of(b * H, H), H)
            q = qabs_s[r, :].astype(BF16)
            s = _dot_nt(q, c) * SCALE
            m = jnp.max(s, axis=-1, keepdims=True)
            p = jnp.exp(s - m)
            l = jnp.sum(p, axis=-1, keepdims=True)
            ctxc_s[r, :] = _dot(p.astype(BF16), c) / l

        def ctx_piece(j, c):
            lhs = jnp.concatenate([ctxc_s[pl.ds(pl.multiple_of(b * H + j * G, G), G), :] for b in range(B)],
                                  axis=0).astype(BF16)
            w = wuv_v[:, pl.ds(pl.multiple_of(j * G, G), G), :].reshape(DC, GW)
            full = _dot(lhs, w)
            mask = gmask()
            parts = [jnp.sum(jnp.where(mask, full[b * G:(b + 1) * G, :], 0.0), axis=0, keepdims=True)
                     for b in range(B)]
            parts.append(jnp.zeros((8 - B, GW), F32))
            ctx_s[:, pl.ds(pl.multiple_of(j * GW, GW), GW)] = jnp.concatenate(parts, axis=0)
            return c

        def out_piece(h, ob):
            return ob + _dot_nt(ctx_s[:, pl.ds(pl.multiple_of(h * DH, DH), DH)].astype(BF16), wob_v[h])

        S = SEGS
        issue(0, S[0])
        c_xb.wait()
        c_xa.wait()
        wait_full(wqb_v, wsem.at[4])
        lax.fori_loop(0, NG // 2, q_piece, 0)
        issue(S[0], S[1])
        lax.fori_loop(NG // 2, NG, q_piece, 0)
        issue(S[1], S[2])
        wait_full(wuk_v, wsem.at[5])
        lax.fori_loop(0, NG // 2, qabs_piece, 0)
        issue(S[2], S[3])
        lax.fori_loop(NG // 2, NG, qabs_piece, 0)

        def attn_iter(b, c):
            for bb in range(B):
                @pl.when(b == bb)
                def _(bb=bb):
                    issue(S[3 + bb], S[4 + bb])
                    wait_full(ckv_v.at[bb], csem.at[bb])
            attn_piece(b)
            return c
        lax.fori_loop(0, B, attn_iter, 0)
        issue(S[7], S[8])
        wait_full(wuv_v, wsem.at[6])
        lax.fori_loop(0, NG // 2, ctx_piece, 0)
        issue(S[8], S[9])
        lax.fori_loop(NG // 2, NG, ctx_piece, 0)
        issue(S[9], S[10])
        wait_full(wob_v, wsem.at[7])
        ob = lax.fori_loop(0, H, out_piece, jnp.zeros((8, DM), F32), unroll=4)
        o_ref[:, DM:2 * DM] = ob[0:B, :].astype(o_ref.dtype)
        issue(S[10], S[11])

        wait_full(wqa_v, wsem.at[1])
        qa = _dot(pad8(xa_v[...]), wqa_v[...])
        qa = qa.astype(BF16).astype(F32)
        for h in range(H):
            qh_s[h] = qa[:, h * DH:(h + 1) * DH]
        acc_s[...] = jnp.zeros_like(acc_s)
        oh_s[...] = jnp.zeros_like(oh_s)
        issue(S[11], len(prog))
        for i in range(LOOK):
            kv_issue(i, (i % B) * H + i // B)
        wait_full(woa_v, wsem.at[2])

        def step(i, carry, mode):
            slot = lax.rem(i, NSLOT)
            h = lax.div(i, B)
            b = lax.rem(i, B)
            if mode != "none":
                n = i + LOOK
                nslot, nbh = lax.rem(n, NSLOT), lax.rem(n, B) * H + lax.div(n, B)
                if mode == "last":
                    kv_issue(nslot, nbh, last_seq, last_prio)
                else:
                    kv_issue(nslot, nbh)
            q = qh_s[h].astype(BF16)
            wait_full(kv.at[slot, 0], kvsem.at[slot, 0])
            s = _dot_nt(q, kv[slot, 0]) * SCALE
            m = jnp.max(s, axis=-1, keepdims=True)
            p = jnp.exp(s - m)
            l = jnp.sum(p, axis=-1, keepdims=True)
            p = p.astype(BF16)
            wait_full(kv.at[slot, 1, pl.ds(0, HALF)], kvsem.at[slot, 1])
            o = _dot(p[:, 0:HALF], kv[slot, 1, 0:HALF, :])
            wait_full(kv.at[slot, 1, pl.ds(HALF, HALF)], kvsem.at[slot, 2])
            o = (o + _dot(p[:, HALF:SK], kv[slot, 1, HALF:SK, :])) / l
            row = lax.broadcasted_iota(jnp.int32, (8, DH), 0)
            oh_s[...] = jnp.where(row == b, o, oh_s[...])

            @pl.when(b == B - 1)
            def _():
                w = woa_v[:, pl.ds(pl.multiple_of(h * DH, DH), DH)]
                acc_s[...] += _dot_nt(oh_s[...].astype(BF16), w)
            return carry

        lax.fori_loop(0, NSTEP - LOOK - 1, functools.partial(step, mode="main"), 0)
        step(NSTEP - LOOK - 1, 0, "last")
        lax.fori_loop(NSTEP - LOOK, NSTEP, functools.partial(step, mode="none"), 0)
        o_ref[:, 0:DM] = acc_s[0:B, :].astype(o_ref.dtype)

    scratch = [
        pltpu.VMEM((B, DM), BF16), pltpu.VMEM((B, DM), BF16),
        pltpu.VMEM((DM, H * DH), BF16), pltpu.VMEM((DM, H * DH), BF16),
        pltpu.VMEM((DM, H, DH), BF16), pltpu.VMEM((DC, H, DH), BF16), pltpu.VMEM((DC, H, DH), BF16),
        pltpu.VMEM((H, DM, DH), BF16), pltpu.VMEM((B, SK, DC), BF16),
        pltpu.VMEM((NSLOT, 2, SK, DH), BF16),
        pltpu.VMEM((H, 8, DH), F32), pltpu.VMEM((8, DH), F32), pltpu.VMEM((8, DM), F32),
        pltpu.VMEM((8, H * DH), F32), pltpu.VMEM((B * H, DC), F32), pltpu.VMEM((B * H, DC), F32),
        pltpu.VMEM((8, H * DH), F32),
        pltpu.SemaphoreType.DMA((8,)), pltpu.SemaphoreType.DMA((B,)),
        pltpu.SemaphoreType.DMA((NSLOT, 3)),
    ]
    return kernel, scratch


@jax.jit
def pallas_concat_heads__mha_block_cached__compressed_kv_cla__decode_kernel(
    A_x, A_k_cache, A_v_cache, A_wq, A_wo, B_x, B_c_kv, B_w_q, B_w_uk, B_w_uv, B_w_o,
):
    kernel, scratch = make_kernel(BS=8)
    args = (
        A_x.reshape(B, DM),
        A_k_cache.reshape(B * H, SK, DH),
        A_v_cache.reshape(B * H, SK, DH),
        A_wq,
        A_wo.T,
        B_x.reshape(B, DM),
        B_c_kv,
        B_w_q, B_w_uk, B_w_uv,
        B_w_o.transpose(0, 2, 1),
    )
    out = pl.pallas_call(
        kernel,
        in_specs=[pl.BlockSpec(memory_space=pltpu.HBM)] * 11,
        out_specs=pl.BlockSpec(memory_space=pltpu.VMEM),
        out_shape=jax.ShapeDtypeStruct((B, 2 * DM), BF16),
        scratch_shapes=scratch,
        compiler_params=pltpu.CompilerParams(vmem_limit_bytes=110 * 1024 * 1024, disable_bounds_checks=True),
    )(*args)
    return out.reshape(B, 1, 2 * DM)
```

```python
import functools
import jax
import jax.numpy as jnp
from jax import lax
import jax.experimental.pallas as pl
import jax.experimental.pallas.tpu as pltpu

B, H, SK, DH, DM, DC = 4, 32, 4096, 128, 576, 512
NSTEP = B * H
F32 = jnp.float32
BF16 = jnp.bfloat16
NT = (((1,), (1,)), ((), ()))
SCALE = float(DH) ** -0.5
G = 8
NG = H // G
GW = G * DH
SUB = 128
HALF = SK // 2
ORDER = ("wqb", "wuk", "ckv0", "ckv1", "ckv2", "ckv3", "wuv", "wob", "wqa", "woa")
NUNITS = dict(wqb=144, wuk=128, ckv0=128, ckv1=128, ckv2=128, ckv3=128, wuv=128, wob=128, wqa=144, woa=144)


def _dot(a, b):
    return jnp.dot(a, b, preferred_element_type=F32)


def _dot_nt(a, b):
    return lax.dot_general(a, b, NT, preferred_element_type=F32)


def streams_seq(lo, hi, S):
    n = hi - lo
    bnd = [lo + round(n * k / S) for k in range(S + 1)]
    pos = bnd[:-1]
    seq = []
    while len(seq) < n:
        for s in range(S):
            if pos[s] < bnd[s + 1]:
                seq.append(pos[s])
                pos[s] += 1
    return seq


def make_kernel(NSLOT=3, KVS=6, KVP=(0, 1, 0), BS=2, BP=(0, 1), LASTS=(3, 2), LASTP=(0, 1, 0), KVSEQ=None, KVPRIO=None,
                SEGS=(272, 336, 400, 464, 528, 656, 784, 912, 1040, 1112, 1184, 1328)):
    LOOK = NSLOT - 1
    kv_seq = list(KVSEQ) if KVSEQ is not None else streams_seq(0, 64, KVS)
    kv_prio = list(KVPRIO) if KVPRIO is not None else [KVP[i % len(KVP)] for i in range(64)]
    last_seq = streams_seq(0, 32, LASTS[0]) + streams_seq(32, 48, LASTS[1]) + streams_seq(48, 64, LASTS[1])
    last_prio = [LASTP[i % len(LASTP)] for i in range(64)]

    def kernel(xa_h, k_h, v_h, wqa_h, woa_h, xb_h, ckv_h, wqb_h, wuk_h, wuv_h, wob_h,
               o_ref,
               xa_v, xb_v, wqa_v, woa_v, wqb_v, wuk_v, wuv_v, wob_v, ckv_v,
               kv, qh_s, oh_s, acc_s, qb_s, qabs_s, ctxc_s, ctx_s, p_s, l_s, o_s,
               wsem, csem, kvsem):

        def unit_refs(name, u):
            if name in ("wqb", "wuk", "wuv"):
                s, d, sem = {"wqb": (wqb_h, wqb_v, wsem.at[4]), "wuk": (wuk_h, wuk_v, wsem.at[5]),
                             "wuv": (wuv_h, wuv_v, wsem.at[6])}[name]
                return s.at[pl.ds(u * 4, 4)], d.at[pl.ds(u * 4, 4)], sem
            if name == "wob":
                h, r = u // 4, (u % 4) * 144
                return wob_h.at[h, pl.ds(r, 144)], wob_v.at[h, pl.ds(r, 144)], wsem.at[7]
            if name in ("wqa", "woa"):
                s, d, sem = {"wqa": (wqa_h, wqa_v, wsem.at[1]), "woa": (woa_h, woa_v, wsem.at[2])}[name]
                r, c = (u // 2) * 8, (u % 2) * 2048
                return s.at[pl.ds(r, 8), pl.ds(c, 2048)], d.at[pl.ds(r, 8), pl.ds(c, 2048)], sem
            b = int(name[3])
            return ckv_h.at[b, pl.ds(u * 32, 32)], ckv_v.at[b, pl.ds(u * 32, 32)], csem.at[b]

        prog = []
        for name in ORDER:
            for u in streams_seq(0, NUNITS[name], BS):
                prog.append((name, u))

        def issue(lo, hi):
            for n in range(lo, hi):
                s, d, sem = unit_refs(*prog[n])
                pltpu.make_async_copy(s, d, sem).start(priority=BP[n % len(BP)])

        def kv_issue(slot, bh, seq=kv_seq, prio=kv_prio):
            for c, pr in zip(seq, prio):
                which, r = c >> 5, (c & 31) * SUB
                src = k_h if which == 0 else v_h
                si = 0 if which == 0 else 1 + r // HALF
                pltpu.make_async_copy(src.at[bh, pl.ds(r, SUB)], kv.at[slot, which, pl.ds(r, SUB)],
                                      kvsem.at[slot, si]).start(priority=pr)

        def wait_full(dst, sem):
            pltpu.make_async_copy(dst, dst, sem).wait()

        c_xa = pltpu.make_async_copy(xa_h, xa_v, wsem.at[0])
        c_xb = pltpu.make_async_copy(xb_h, xb_v, wsem.at[3])
        c_xb.start()
        c_xa.start()

        def pad8(x):
            return jnp.concatenate([x.astype(F32), jnp.zeros((8 - B, x.shape[1]), F32)], axis=0).astype(BF16)

        def gmask():
            rows = lax.broadcasted_iota(jnp.int32, (G, GW), 0)
            cols = lax.broadcasted_iota(jnp.int32, (G, GW), 1) // DH
            return rows == cols

        def q_piece(j, c):
            w = wqb_v[:, pl.ds(pl.multiple_of(j * G, G), G), :].reshape(DM, GW)
            qb_s[:, pl.ds(pl.multiple_of(j * GW, GW), GW)] = _dot(pad8(xb_v[...]), w).astype(BF16).astype(F32)
            return c

        def qabs_piece(j, c):
            qg = qb_s[:, pl.ds(pl.multiple_of(j * GW, GW), GW)]
            mask = gmask()
            parts = [jnp.where(mask, jnp.broadcast_to(qg[b:b + 1, :], (G, GW)), 0.0) for b in range(B)]
            qexp = jnp.concatenate(parts, axis=0).astype(BF16)
            w = wuk_v[:, pl.ds(pl.multiple_of(j * G, G), G), :].reshape(DC, GW)
            res = _dot_nt(qexp, w)
            for b in range(B):
                qabs_s[pl.ds(pl.multiple_of(b * H + j * G, G), G), :] = res[b * G:(b + 1) * G, :]
            return c

        def attn_piece(b):
            c = ckv_v[b]
            r = pl.ds(pl.multiple_of(b * H, H), H)
            q = qabs_s[r, :].astype(BF16)
            s = _dot_nt(q, c) * SCALE
            m = jnp.max(s, axis=-1, keepdims=True)
            p = jnp.exp(s - m)
            l = jnp.sum(p, axis=-1, keepdims=True)
            ctxc_s[r, :] = _dot(p.astype(BF16), c) / l

        def ctx_piece(j, c):
            lhs = jnp.concatenate([ctxc_s[pl.ds(pl.multiple_of(b * H + j * G, G), G), :] for b in range(B)],
                                  axis=0).astype(BF16)
            w = wuv_v[:, pl.ds(pl.multiple_of(j * G, G), G), :].reshape(DC, GW)
            full = _dot(lhs, w)
            mask = gmask()
            parts = [jnp.sum(jnp.where(mask, full[b * G:(b + 1) * G, :], 0.0), axis=0, keepdims=True)
                     for b in range(B)]
            parts.append(jnp.zeros((8 - B, GW), F32))
            ctx_s[:, pl.ds(pl.multiple_of(j * GW, GW), GW)] = jnp.concatenate(parts, axis=0)
            return c

        def out_piece(h, ob):
            return ob + _dot_nt(ctx_s[:, pl.ds(pl.multiple_of(h * DH, DH), DH)].astype(BF16), wob_v[h])

        S = SEGS
        issue(0, S[0])
        c_xb.wait()
        c_xa.wait()
        wait_full(wqb_v, wsem.at[4])
        lax.fori_loop(0, NG // 2, q_piece, 0)
        issue(S[0], S[1])
        lax.fori_loop(NG // 2, NG, q_piece, 0)
        issue(S[1], S[2])
        wait_full(wuk_v, wsem.at[5])
        lax.fori_loop(0, NG // 2, qabs_piece, 0)
        issue(S[2], S[3])
        lax.fori_loop(NG // 2, NG, qabs_piece, 0)

        def attn_iter(b, c):
            for bb in range(B):
                @pl.when(b == bb)
                def _(bb=bb):
                    issue(S[3 + bb], S[4 + bb])
                    wait_full(ckv_v.at[bb], csem.at[bb])
            attn_piece(b)
            return c
        lax.fori_loop(0, B, attn_iter, 0)
        issue(S[7], S[8])
        wait_full(wuv_v, wsem.at[6])
        lax.fori_loop(0, NG // 2, ctx_piece, 0)
        issue(S[8], S[9])
        lax.fori_loop(NG // 2, NG, ctx_piece, 0)
        issue(S[9], S[10])
        wait_full(wob_v, wsem.at[7])
        ob = lax.fori_loop(0, H, out_piece, jnp.zeros((8, DM), F32), unroll=4)
        o_ref[:, DM:2 * DM] = ob[0:B, :].astype(o_ref.dtype)
        issue(S[10], S[11])

        wait_full(wqa_v, wsem.at[1])
        qa = _dot(pad8(xa_v[...]), wqa_v[...])
        qa = qa.astype(BF16).astype(F32)
        for h in range(H):
            qh_s[h] = qa[:, h * DH:(h + 1) * DH]
        acc_s[...] = jnp.zeros_like(acc_s)
        oh_s[...] = jnp.zeros_like(oh_s)
        issue(S[11], len(prog))
        for i in range(LOOK):
            kv_issue(i, (i % B) * H + i // B)
        wait_full(woa_v, wsem.at[2])

        def step(i, carry, mode, split=False):
            slot = lax.rem(i, NSLOT)
            h = lax.div(i, B)
            b = lax.rem(i, B)
            if mode != "none":
                n = i + LOOK
                nslot, nbh = lax.rem(n, NSLOT), lax.rem(n, B) * H + lax.div(n, B)
                if mode == "last":
                    kv_issue(nslot, nbh, last_seq, last_prio)
                else:
                    kv_issue(nslot, nbh)
            q = qh_s[h].astype(BF16)
            wait_full(kv.at[slot, 0], kvsem.at[slot, 0])
            if not split:
                wait_full(kv.at[slot, 1, pl.ds(0, HALF)], kvsem.at[slot, 1])
                wait_full(kv.at[slot, 1, pl.ds(HALF, HALF)], kvsem.at[slot, 2])
            s = _dot_nt(q, kv[slot, 0]) * SCALE
            m = jnp.max(s, axis=-1, keepdims=True)
            p = jnp.exp(s - m)
            l = jnp.sum(p, axis=-1, keepdims=True)
            p = p.astype(BF16)
            if split:
                p_s[...] = p
                l_s[...] = jnp.broadcast_to(l, l_s.shape)
                wait_full(kv.at[slot, 1, pl.ds(0, HALF)], kvsem.at[slot, 1])
                o_s[...] = _dot(p_s[:, 0:HALF], kv[slot, 1, 0:HALF, :])
                wait_full(kv.at[slot, 1, pl.ds(HALF, HALF)], kvsem.at[slot, 2])
                o = (o_s[...] + _dot(p_s[:, HALF:SK], kv[slot, 1, HALF:SK, :])) / l_s[...]
            else:
                o = _dot(p, kv[slot, 1]) / l
            row = lax.broadcasted_iota(jnp.int32, (8, DH), 0)
            oh_s[...] = jnp.where(row == b, o, oh_s[...])

            @pl.when(b == B - 1)
            def _():
                w = woa_v[:, pl.ds(pl.multiple_of(h * DH, DH), DH)]
                acc_s[...] += _dot_nt(oh_s[...].astype(BF16), w)
            return carry

        lax.fori_loop(0, NSTEP - LOOK - 1, functools.partial(step, mode="main"), 0)
        step(jnp.int32(NSTEP - LOOK - 1), 0, "last")
        if LOOK > 1:
            lax.fori_loop(NSTEP - LOOK, NSTEP - 1, functools.partial(step, mode="none"), 0)
        step(jnp.int32(NSTEP - 1), 0, "none", split=True)
        o_ref[:, 0:DM] = acc_s[0:B, :].astype(o_ref.dtype)

    scratch = [
        pltpu.VMEM((B, DM), BF16), pltpu.VMEM((B, DM), BF16),
        pltpu.VMEM((DM, H * DH), BF16), pltpu.VMEM((DM, H * DH), BF16),
        pltpu.VMEM((DM, H, DH), BF16), pltpu.VMEM((DC, H, DH), BF16), pltpu.VMEM((DC, H, DH), BF16),
        pltpu.VMEM((H, DM, DH), BF16), pltpu.VMEM((B, SK, DC), BF16),
        pltpu.VMEM((NSLOT, 2, SK, DH), BF16),
        pltpu.VMEM((H, 8, DH), F32), pltpu.VMEM((8, DH), F32), pltpu.VMEM((8, DM), F32),
        pltpu.VMEM((8, H * DH), F32), pltpu.VMEM((B * H, DC), F32), pltpu.VMEM((B * H, DC), F32),
        pltpu.VMEM((8, H * DH), F32),
        pltpu.VMEM((8, SK), BF16), pltpu.VMEM((8, DH), F32), pltpu.VMEM((8, DH), F32),
        pltpu.SemaphoreType.DMA((8,)), pltpu.SemaphoreType.DMA((B,)),
        pltpu.SemaphoreType.DMA((NSLOT, 3)),
    ]
    return kernel, scratch


@jax.jit
def pallas_concat_heads__mha_block_cached__compressed_kv_cla__decode_kernel(
    A_x, A_k_cache, A_v_cache, A_wq, A_wo, B_x, B_c_kv, B_w_q, B_w_uk, B_w_uv, B_w_o,
):
    kernel, scratch = make_kernel(BS=8, LASTP=(1, 1))
    args = (
        A_x.reshape(B, DM),
        A_k_cache.reshape(B * H, SK, DH),
        A_v_cache.reshape(B * H, SK, DH),
        A_wq,
        A_wo.T,
        B_x.reshape(B, DM),
        B_c_kv,
        B_w_q, B_w_uk, B_w_uv,
        B_w_o.transpose(0, 2, 1),
    )
    out = pl.pallas_call(
        kernel,
        in_specs=[pl.BlockSpec(memory_space=pltpu.HBM)] * 11,
        out_specs=pl.BlockSpec(memory_space=pltpu.VMEM),
        out_shape=jax.ShapeDtypeStruct((B, 2 * DM), BF16),
        scratch_shapes=scratch,
        compiler_params=pltpu.CompilerParams(vmem_limit_bytes=110 * 1024 * 1024, disable_bounds_checks=True),
    )(*args)
    return out.reshape(B, 1, 2 * DM)
```

```python
import jax
import jax.numpy as jnp
from jax import lax
import jax.experimental.pallas as pl
import jax.experimental.pallas.tpu as pltpu

B, H, SK, DH, DM, DC = 4, 32, 4096, 128, 576, 512
NSTEP = B * H
F32 = jnp.float32
BF16 = jnp.bfloat16
NT = (((1,), (1,)), ((), ()))
SCALE = float(DH) ** -0.5
G = 8
NG = H // G
GW = G * DH
SUB = 128
HALF = SK // 2
BS = 8
ORDER = ("wqb", "wuk", "ckv0", "ckv1", "ckv2", "ckv3", "wuv", "wob", "wqa", "woa")
NUNITS = dict(wqb=144, wuk=128, ckv0=128, ckv1=128, ckv2=128, ckv3=128, wuv=128, wob=144, wqa=144, woa=144)


def _dot(a, b):
    return jnp.dot(a, b, preferred_element_type=F32)


def _dot_nt(a, b):
    return lax.dot_general(a, b, NT, preferred_element_type=F32)


def _streams(lo, hi, n_streams):
    n = hi - lo
    bnd = [lo + round(n * k / n_streams) for k in range(n_streams + 1)]
    pos = bnd[:-1]
    seq = []
    while len(seq) < n:
        for s in range(n_streams):
            if pos[s] < bnd[s + 1]:
                seq.append(pos[s])
                pos[s] += 1
    return seq


def make_kernel(NSLOT=3, KVS=6, KVP=(0, 1, 0), LASTS=(3, 2), LASTP=(1, 1), OUT_UNROLL=4,
                SEGS=(272, 336, 400, 464, 528, 656, 784, 912, 1056, 1128, 1200, 1344)):
    LOOK = NSLOT - 1
    kv_seq = _streams(0, 64, KVS)
    kv_prio = [KVP[i % len(KVP)] for i in range(64)]
    last_seq = _streams(0, 32, LASTS[0]) + _streams(32, 48, LASTS[1]) + _streams(48, 64, LASTS[1])
    last_prio = [LASTP[i % len(LASTP)] for i in range(64)]

    def kernel(xa_h, k_h, v_h, wqa_h, woa_h, xb_h, ckv_h, wqb_h, wuk_h, wuv_h, wob_h,
               o_ref,
               xa_v, xb_v, wqa_v, woa_v, wqb_v, wuk_v, wuv_v, wob_v, ckv_v,
               kv, qh_s, oh_s, acc_s, qb_s, qabs_s, ctxc_s, ctx_s, p_s, l_s, o_s,
               wsem, csem, kvsem):

        def unit_refs(name, u):
            if name in ("wqb", "wuk", "wuv"):
                s, d, sem = {"wqb": (wqb_h, wqb_v, wsem.at[4]), "wuk": (wuk_h, wuk_v, wsem.at[5]),
                             "wuv": (wuv_h, wuv_v, wsem.at[6])}[name]
                return s.at[pl.ds(u * 4, 4)], d.at[pl.ds(u * 4, 4)], sem
            if name == "wob":
                r = pl.ds(pl.multiple_of(u * SUB, SUB), SUB)
                return wob_h.at[r], wob_v.at[r], wsem.at[7]
            if name in ("wqa", "woa"):
                s, d, sem = {"wqa": (wqa_h, wqa_v, wsem.at[1]), "woa": (woa_h, woa_v, wsem.at[2])}[name]
                r = pl.ds(pl.multiple_of(lax.div(u, 2) * 8, 8), 8)
                c = pl.ds(pl.multiple_of(lax.rem(u, 2) * 2048, 2048), 2048)
                return s.at[r, c], d.at[r, c], sem
            b = int(name[3])
            r = pl.ds(pl.multiple_of(u * 32, 32), 32)
            return ckv_h.at[b, r], ckv_v.at[b, r], csem.at[b]

        def issue(lo, hi):
            base = 0
            for name in ORDER:
                n = NUNITS[name]
                a, b = max(lo, base) - base, min(hi, base + n) - base
                if b > a:
                    assert a % BS == 0 and b % BS == 0

                    def body(p, c, name=name, n=n):
                        for s in range(BS):
                            src, dst, sem = unit_refs(name, s * (n // BS) + p)
                            pltpu.make_async_copy(src, dst, sem).start(priority=s % 2)
                        return c
                    lax.fori_loop(a // BS, b // BS, body, 0)
                base += n

        def kv_issue(slot, bh, seq, prio):
            for c, pr in zip(seq, prio):
                which, r = c >> 5, (c & 31) * SUB
                src = k_h if which == 0 else v_h
                si = 0 if which == 0 else 1 + r // HALF
                pltpu.make_async_copy(src.at[bh, pl.ds(r, SUB)], kv.at[slot, which, pl.ds(r, SUB)],
                                      kvsem.at[slot, si]).start(priority=pr)

        def wait_full(dst, sem):
            pltpu.make_async_copy(dst, dst, sem).wait()

        c_xa = pltpu.make_async_copy(xa_h, xa_v, wsem.at[0])
        c_xb = pltpu.make_async_copy(xb_h, xb_v, wsem.at[3])
        c_xb.start()
        c_xa.start()

        def pad8(x):
            return jnp.concatenate([x.astype(F32), jnp.zeros((8 - B, x.shape[1]), F32)], axis=0).astype(BF16)

        def gmask():
            rows = lax.broadcasted_iota(jnp.int32, (G, GW), 0)
            cols = lax.broadcasted_iota(jnp.int32, (G, GW), 1) // DH
            return rows == cols

        def q_piece(j):
            w = wqb_v[:, pl.ds(pl.multiple_of(j * G, G), G), :].reshape(DM, GW)
            qb_s[:, pl.ds(pl.multiple_of(j * GW, GW), GW)] = _dot(pad8(xb_v[...]), w).astype(BF16).astype(F32)

        def qabs_piece(j):
            qg = qb_s[:, pl.ds(pl.multiple_of(j * GW, GW), GW)]
            mask = gmask()
            parts = [jnp.where(mask, jnp.broadcast_to(qg[b:b + 1, :], (G, GW)), 0.0) for b in range(B)]
            qexp = jnp.concatenate(parts, axis=0).astype(BF16)
            w = wuk_v[:, pl.ds(pl.multiple_of(j * G, G), G), :].reshape(DC, GW)
            res = _dot_nt(qexp, w)
            for b in range(B):
                qabs_s[pl.ds(pl.multiple_of(b * H + j * G, G), G), :] = res[b * G:(b + 1) * G, :]

        def attn_piece(b):
            c = ckv_v[b]
            r = pl.ds(pl.multiple_of(b * H, H), H)
            q = qabs_s[r, :].astype(BF16)
            s = _dot_nt(q, c) * SCALE
            m = jnp.max(s, axis=-1, keepdims=True)
            p = jnp.exp(s - m)
            l = jnp.sum(p, axis=-1, keepdims=True)
            ctxc_s[r, :] = _dot(p.astype(BF16), c) / l

        def ctx_piece(j):
            lhs = jnp.concatenate([ctxc_s[pl.ds(pl.multiple_of(b * H + j * G, G), G), :] for b in range(B)],
                                  axis=0).astype(BF16)
            w = wuv_v[:, pl.ds(pl.multiple_of(j * G, G), G), :].reshape(DC, GW)
            full = _dot(lhs, w)
            mask = gmask()
            parts = [jnp.sum(jnp.where(mask, full[b * G:(b + 1) * G, :], 0.0), axis=0, keepdims=True)
                     for b in range(B)]
            parts.append(jnp.zeros((8 - B, GW), F32))
            ctx_s[:, pl.ds(pl.multiple_of(j * GW, GW), GW)] = jnp.concatenate(parts, axis=0)

        def out_piece(h, ob):
            w = wob_v[pl.ds(pl.multiple_of(h * DM, 16), DM), :]
            return ob + _dot_nt(ctx_s[:, pl.ds(pl.multiple_of(h * DH, DH), DH)].astype(BF16), w)

        def grouped(piece, lo, hi):
            def body(j, c):
                @pl.when(j == NG // 2)
                def _():
                    issue(lo, hi)
                piece(j)
                return c
            lax.fori_loop(0, NG, body, 0)

        S = SEGS
        issue(0, S[0])
        c_xb.wait()
        c_xa.wait()
        wait_full(wqb_v, wsem.at[4])
        grouped(q_piece, S[0], S[1])
        issue(S[1], S[2])
        wait_full(wuk_v, wsem.at[5])
        grouped(qabs_piece, S[2], S[3])

        def attn_iter(b, c):
            for bb in range(B):
                @pl.when(b == bb)
                def _(bb=bb):
                    issue(S[3 + bb], S[4 + bb])
                    wait_full(ckv_v.at[bb], csem.at[bb])
            attn_piece(b)
            return c
        lax.fori_loop(0, B, attn_iter, 0)
        issue(S[7], S[8])
        wait_full(wuv_v, wsem.at[6])
        grouped(ctx_piece, S[8], S[9])
        issue(S[9], S[10])
        wait_full(wob_v, wsem.at[7])
        ob = lax.fori_loop(0, H, out_piece, jnp.zeros((8, DM), F32), unroll=OUT_UNROLL)
        o_ref[:, DM:2 * DM] = ob[0:B, :].astype(o_ref.dtype)
        issue(S[10], S[11])

        wait_full(wqa_v, wsem.at[1])
        qa = _dot(pad8(xa_v[...]), wqa_v[...])
        qa = qa.astype(BF16).astype(F32)
        for h in range(H):
            qh_s[h] = qa[:, h * DH:(h + 1) * DH]
        acc_s[...] = jnp.zeros_like(acc_s)
        oh_s[...] = jnp.zeros_like(oh_s)
        issue(S[11], sum(NUNITS.values()))
        for i in range(LOOK):
            kv_issue(i, (i % B) * H + i // B, kv_seq, kv_prio)
        wait_full(woa_v, wsem.at[2])

        def step(i, final):
            slot = lax.rem(i, NSLOT)
            h = lax.div(i, B)
            b = lax.rem(i, B)
            if not final:
                n = i + LOOK
                nslot, nbh = lax.rem(n, NSLOT), lax.rem(n, B) * H + lax.div(n, B)

                @pl.when(n < NSTEP - 1)
                def _():
                    kv_issue(nslot, nbh, kv_seq, kv_prio)

                @pl.when(n == NSTEP - 1)
                def _():
                    kv_issue(nslot, nbh, last_seq, last_prio)
            q = qh_s[h].astype(BF16)
            wait_full(kv.at[slot, 0], kvsem.at[slot, 0])
            if not final:
                wait_full(kv.at[slot, 1, pl.ds(0, HALF)], kvsem.at[slot, 1])
                wait_full(kv.at[slot, 1, pl.ds(HALF, HALF)], kvsem.at[slot, 2])
            s = _dot_nt(q, kv[slot, 0]) * SCALE
            m = jnp.max(s, axis=-1, keepdims=True)
            p = jnp.exp(s - m)
            l = jnp.sum(p, axis=-1, keepdims=True)
            p = p.astype(BF16)
            if final:
                p_s[...] = p
                l_s[...] = jnp.broadcast_to(l, l_s.shape)
                wait_full(kv.at[slot, 1, pl.ds(0, HALF)], kvsem.at[slot, 1])
                o_s[...] = _dot(p_s[:, 0:HALF], kv[slot, 1, 0:HALF, :])
                wait_full(kv.at[slot, 1, pl.ds(HALF, HALF)], kvsem.at[slot, 2])
                o = (o_s[...] + _dot(p_s[:, HALF:SK], kv[slot, 1, HALF:SK, :])) / l_s[...]
            else:
                o = _dot(p, kv[slot, 1]) / l
            row = lax.broadcasted_iota(jnp.int32, (8, DH), 0)
            oh_s[...] = jnp.where(row == b, o, oh_s[...])

            @pl.when(b == B - 1)
            def _():
                w = woa_v[:, pl.ds(pl.multiple_of(h * DH, DH), DH)]
                acc_s[...] += _dot_nt(oh_s[...].astype(BF16), w)

        def loop_body(i, c):
            step(i, False)
            return c
        lax.fori_loop(0, NSTEP - 1, loop_body, 0)
        step(jnp.int32(NSTEP - 1), True)
        o_ref[:, 0:DM] = acc_s[0:B, :].astype(o_ref.dtype)

    scratch = [
        pltpu.VMEM((B, DM), BF16), pltpu.VMEM((B, DM), BF16),
        pltpu.VMEM((DM, H * DH), BF16), pltpu.VMEM((DM, H * DH), BF16),
        pltpu.VMEM((DM, H, DH), BF16), pltpu.VMEM((DC, H, DH), BF16), pltpu.VMEM((DC, H, DH), BF16),
        pltpu.VMEM((H * DM, DH), BF16), pltpu.VMEM((B, SK, DC), BF16),
        pltpu.VMEM((NSLOT, 2, SK, DH), BF16),
        pltpu.VMEM((H, 8, DH), F32), pltpu.VMEM((8, DH), F32), pltpu.VMEM((8, DM), F32),
        pltpu.VMEM((8, H * DH), F32), pltpu.VMEM((B * H, DC), F32), pltpu.VMEM((B * H, DC), F32),
        pltpu.VMEM((8, H * DH), F32),
        pltpu.VMEM((8, SK), BF16), pltpu.VMEM((8, DH), F32), pltpu.VMEM((8, DH), F32),
        pltpu.SemaphoreType.DMA((8,)), pltpu.SemaphoreType.DMA((B,)),
        pltpu.SemaphoreType.DMA((NSLOT, 3)),
    ]
    return kernel, scratch


@jax.jit
def pallas_concat_heads__mha_block_cached__compressed_kv_cla__decode_kernel(
    A_x, A_k_cache, A_v_cache, A_wq, A_wo, B_x, B_c_kv, B_w_q, B_w_uk, B_w_uv, B_w_o,
):
    kernel, scratch = make_kernel()
    args = (
        A_x.reshape(B, DM),
        A_k_cache.reshape(B * H, SK, DH),
        A_v_cache.reshape(B * H, SK, DH),
        A_wq,
        A_wo.T,
        B_x.reshape(B, DM),
        B_c_kv,
        B_w_q, B_w_uk, B_w_uv,
        B_w_o.transpose(0, 2, 1).reshape(H * DM, DH),
    )
    out = pl.pallas_call(
        kernel,
        in_specs=[pl.BlockSpec(memory_space=pltpu.HBM)] * 11,
        out_specs=pl.BlockSpec(memory_space=pltpu.VMEM),
        out_shape=jax.ShapeDtypeStruct((B, 2 * DM), BF16),
        scratch_shapes=scratch,
        compiler_params=pltpu.CompilerParams(vmem_limit_bytes=110 * 1024 * 1024),
    )(*args)
    return out.reshape(B, 1, 2 * DM)
```
